```python
import os as _os
_os.environ.setdefault("JAX_PLATFORMS", "cpu")
import jax
import jax.numpy as jnp

def _softmax(x, axis=-1):
    return jax.nn.softmax(x, axis=axis)
def _gelu(x):
    return jax.nn.gelu(x, approximate=True)
def _silu(x):
    return jax.nn.silu(x)
def _sigmoid(x):
    return jax.nn.sigmoid(x)
def _layernorm(x, axis=-1, eps=1e-5):
    m = jnp.mean(x, axis=axis, keepdims=True)
    v = jnp.var(x, axis=axis, keepdims=True)
    return (x - m) / jnp.sqrt(v + eps)
def _scatter_add(tgt, idx, src, axis=0):
    return tgt.at[idx].add(src)
def _segment_sum(src, seg, n):
    return jax.ops.segment_sum(src, seg, n)
class _Rng:
    def __init__(self, key):
        self._k = key
    def _next(self):
        self._k, sub = jax.random.split(self._k)
        return sub
    def normal(self, shape):
        return jax.random.normal(self._next(), shape, dtype=jnp.bfloat16)
    def randint(self, lo, hi, shape):
        return jax.random.randint(self._next(), shape, lo, hi, dtype=jnp.int32)
    def uniform(self, shape, lo=0.0, hi=1.0):
        return jax.random.uniform(self._next(), shape, jnp.bfloat16, lo, hi)
    def permutation(self, n):
        return jax.random.permutation(self._next(), n)


kernel_name = 'parallel_sum__sliding_block__moe_arch_mod__prompt'

def setup_inputs():
    _rng = _Rng(jax.random.key(int.from_bytes(__import__("os").urandom(4), "little")))
    _w = (lambda a: (lambda t: t.astype(jnp.bfloat16) if jnp.issubdtype(t.dtype, jnp.floating) else t)(jnp.asarray(a)))
    def _A_setup():
        B, S, D = 1, 2048, 512
        return {
            "x": _w((lambda *s: _rng.normal(s) * 0.05)(B, S, D)),
            "wqkv": _w((lambda *s: _rng.normal(s) * 0.05)(D, 3 * D)),
            "wo": _w((lambda *s: _rng.normal(s) * 0.05)(D, D)),
        }
    _A_in = _A_setup()

    def _B_setup():
        B, S, D, F, C = 1, 2048, 512, 1376, 1
        return {
            "x": _w((lambda *s: _rng.normal(s) * 0.05)(B, S, D)),
            "w_r": _w((lambda *s: _rng.normal(s) * 0.05)(D)),
            "w_gate": _w((lambda *s: _rng.normal(s) * 0.05)(D, F)),
            "w_up": _w((lambda *s: _rng.normal(s) * 0.05)(D, F)),
            "w_down": _w((lambda *s: _rng.normal(s) * 0.05)(F, D)),
        }
    _B_in = _B_setup()

    return {
        "A_x": _A_in["x"],
        "A_wqkv": _A_in["wqkv"],
        "A_wo": _A_in["wo"],
        "B_x": _B_in["x"],
        "B_w_r": _B_in["w_r"],
        "B_w_gate": _B_in["w_gate"],
        "B_w_up": _B_in["w_up"],
        "B_w_down": _B_in["w_down"],
    }

def reference(A_x, A_wqkv, A_wo, B_x, B_w_r, B_w_gate, B_w_up, B_w_down):
    def _A_ref(x, wqkv, wo):
        B, S, D = x.shape
        H = 32; Dh = D // H; W = 256
        qkv = (lambda x, *d: x.transpose(*d))((x @ wqkv).reshape(B, S, 3, H, Dh), 2, 0, 3, 1, 4)
        q, k, v = qkv[0], qkv[1], qkv[2]
        scores = jnp.einsum("bhqd,bhkd->bhqk", q, k) * (Dh ** -0.5)
        idx = jnp.arange(S)
        mask = (idx[:, None] - idx[None, :] >= 0) & (idx[:, None] - idx[None, :] < W)
        scores = jnp.where(mask[None, None], scores, -1e9)
        p = _softmax(scores, axis=-1)
        o = jnp.einsum("bhqk,bhkd->bhqd", p, v)
        return (lambda x, *d: x.transpose(*d))(o, 0, 2, 1, 3).reshape(B, S, D) @ wo

    def _B_ref(x, w_r, w_gate, w_up, w_down):
        B, S, D = x.shape
        C = 1
        r = x @ w_r
        idx = jnp.argsort(-r, axis=-1)[:, :C]
        idx_e = jnp.repeat(idx.reshape(B, C, 1), D, axis=2)
        x_sel = jnp.take_along_axis(x, idx_e, axis=1)
        g = _silu(x_sel @ w_gate)
        u = x_sel @ w_up
        y = (g * u) @ w_down
        r_sel = _sigmoid(jnp.take_along_axis(r, idx, axis=1))
        y = y * r_sel.reshape(B, C, 1)
        b_off = (jnp.arange(B) * S).reshape(B, 1)
        flat_idx = (idx + b_off).reshape(B * C)
        zero = (x * 0.0).reshape(B * S, D)
        upd = _scatter_add(zero, flat_idx, y.reshape(B * C, D), axis=0)
        return x + upd.reshape(B, S, D)

    x = A_x
    xn = _layernorm(x, axis=-1)
    return x + _A_ref(xn, A_wqkv, A_wo) + _B_ref(xn, B_w_r, B_w_gate, B_w_up, B_w_down)
```

```python
import functools
ORDER = [int(c, 16) for c in '89ab01234567']
SPLITDOT = int('0')
P3N = int('1')
RESP = int('3')
SLABS = [int(c) for c in '012']
NF = 11
FSLOTS = [int(c) for c in '0']
FSTART = int('0')
CHECK = int('1')
FORCE_SAFE = bool(int('0'))
L_LO = (127 - 40) << 23
L_HI = (127 + 40) << 23
P3U = int('8')
LOOKAHEAD = int('1')
import jax
import jax.numpy as jnp
import numpy as np
from jax import lax
import jax.experimental.pallas as pl
import jax.experimental.pallas.tpu as pltpu

S = 2048
D = 512
F = 1376
T1 = int('512')
N1 = S // T1
NQ = S // 128
LOG2E = 1.4426950408889634
QSCALE = 0.25 * LOG2E
G = 8
B = 128 // G
NR = 256 + B
LG = 3
NU = 8 // G
OPD = 1
T3 = 128
CUTS = (0, 96, 192, NR)
BF = jnp.bfloat16
F32 = jnp.float32
I32 = jnp.int32
NT = (((1,), (1,)), ((), ()))
TN = (((0,), (0,)), ((), ()))


def _np_bf16(v):
    u = np.array([v], np.float32).view(np.uint32)
    u = (u + 0x7FFF + ((u >> 16) & 1)) & 0xFFFF0000
    return float(u.astype(np.uint32).view(np.float32)[0])


EPS_B = _np_bf16(1e-5)


def bi(x):
    return pltpu.bitcast(x, I32)


def bb(x):
    return pltpu.bitcast(x, BF)


def _rb(x):
    return x.astype(BF).astype(F32)


def _kernel(x_hbm, wqkv_hbm, wo_hbm, wr_ref, wg_hbm, wu_hbm, wd_hbm, out_hbm,
            x_v, wqkv_v, wo_v, wg_v, wu_v, wd_v,
            mb_v, ri_v, cs_v, res_v, upd_v, k_v, qt_v, vt_v, pbuf, bias_v, ot_v, on_v, out_v,
            x_sem, w_sem, o_sem):
    XCH = [(0, T1), (T1, T1), (2 * T1, S - 2 * T1)]

    def x_copy(j):
        r = pl.ds(*XCH[j])
        return pltpu.make_async_copy(x_hbm.at[r], x_v.at[r], x_sem.at[j])

    def wq_copy(j):
        c = pl.ds(j * D, D)
        return pltpu.make_async_copy(wqkv_hbm.at[:, c], wqkv_v.at[:, c], w_sem.at[j])

    wo_copy = pltpu.make_async_copy(wo_hbm, wo_v, w_sem.at[3])
    ffn_copies = [
        pltpu.make_async_copy(wg_hbm, wg_v, w_sem.at[4]),
        pltpu.make_async_copy(wu_hbm, wu_v, w_sem.at[5]),
        pltpu.make_async_copy(wd_hbm, wd_v, w_sem.at[6]),
    ]
    x_copy(0).start()
    for j in SLABS:
        wq_copy(j).start()
    x_copy(1).start()

    wr = wr_ref[...].astype(F32).reshape(1, D)
    ki = k_v.bitcast(I32)
    qti = qt_v.bitcast(I32)
    pbi = pbuf.bitcast(I32)
    vti = vt_v.bitcast(I32)

    swr = jnp.sum(wr, axis=1, keepdims=True)

    def row_stats(x):
        mean = jnp.mean(x, axis=1, keepdims=True)
        c = x - mean
        var = jnp.mean(c * c, axis=1, keepdims=True)
        mb = _rb(mean)
        sd = _rb(jnp.sqrt(_rb(_rb(var) + EPS_B)))
        return mb, sd

    def stats(i, best_m, best_i):
        r0 = i * T1 if isinstance(i, int) else pl.multiple_of(i * T1, T1)
        r = pl.ds(r0, T1)
        x = x_v[r, :].astype(F32)
        mb, sd = row_stats(x)
        ri = 1.0 / sd
        mb_v[r, :] = jnp.broadcast_to(mb * ri, (T1, 128))
        ri_v[r, :] = jnp.broadcast_to(ri, (T1, 128))
        rr = _rb((jnp.sum(x * wr, axis=1, keepdims=True) - mb * swr) * ri)
        m = jnp.max(rr, axis=0, keepdims=True)
        rows = lax.broadcasted_iota(I32, (T1, 1), 0) + r0
        idx = jnp.min(jnp.where(rr == m, rows, S), axis=0, keepdims=True)
        better = m > best_m
        return jnp.where(better, m, best_m), jnp.where(better, idx, best_i)

    def colsum(ns):
        for n in ns:
            cs_v[n] = jnp.dot(jnp.ones((16, D), BF), wqkv_v[:, n * 128:(n + 1) * 128],
                              preferred_element_type=F32)[0:8]

    def project(i, ns):
        r0 = i * T1 if isinstance(i, int) else pl.multiple_of(i * T1, T1)
        r = pl.ds(r0, T1)
        accs = {n: jnp.dot(x_v[r, :], wqkv_v[:, n * 128:(n + 1) * 128], preferred_element_type=F32) for n in ns}
        mb = mb_v[r, :]
        ri = ri_v[r, :]
        for n in ns:
            cs = jnp.broadcast_to(cs_v[n, 0:1, :], (T1, 128))
            y = accs[n] * ri - mb * cs
            if n < 4:
                y = y * QSCALE
                for j in range(T1 // 128):
                    qt_v[i * (T1 // 128) + j, n * 128:(n + 1) * 128, :] = y[j * 128:(j + 1) * 128].T.astype(BF)
            elif n < 8:
                k_v[n - 4, r, :] = y.astype(BF)
            else:
                for j in range(T1 // 128):
                    vt_v[i * (T1 // 128) + j, (n - 8) * 128:(n - 7) * 128, :] = y[j * 128:(j + 1) * 128].T.astype(BF)

    x_copy(0).wait()
    carry = stats(0, jnp.full((1, 1), -jnp.inf, F32), jnp.full((1, 1), S - 1, I32))
    for t, j in enumerate(SLABS):
        wq_copy(j).wait()
        if t == 0:
            x_copy(2).start()
            wo_copy.start()
        if t == 2:
            x_copy(1).wait()
        ns = list(range(4 * j, 4 * j + 4))
        colsum(ns)
        project(0, ns)
    carry = stats(1, *carry)

    def p1_body(i, carry):
        @pl.when(i == 1)
        def _():
            x_copy(2).wait()
            for c in ffn_copies:
                c.start()
        project(i, ORDER)
        return stats(jnp.minimum(i + 1, N1 - 1), *carry)

    best_m, best_i = lax.fori_loop(1, N1, p1_body, carry)

    idx = jnp.clip(jnp.max(best_i), 0, S - 1)
    blk = pl.multiple_of((idx // 16) * 16, 16)
    row_sel = lax.broadcasted_iota(I32, (16, 1), 0) == (idx - blk)
    xr = x_v[pl.ds(blk, 16), :].astype(F32)
    mbr, sdr = row_stats(xr)
    xs = jnp.where(row_sel, _rb(xr - mbr) / sdr, 0.0).astype(BF)
    for c in ffn_copies:
        c.wait()
    wo_copy.wait()
    ffn = {}

    def ffn_gate(n):
        r = pl.ds(n * 128, min(128, F - n * 128))
        ffn['g', n] = _rb(lax.dot_general(xs, wg_v[r, :], NT, preferred_element_type=F32))

    def ffn_up(n):
        r = pl.ds(n * 128, min(128, F - n * 128))
        u_ = _rb(lax.dot_general(xs, wu_v[r, :], NT, preferred_element_type=F32))
        g_ = ffn['g', n]
        sg = _rb(g_ * _rb(jax.nn.sigmoid(g_)))
        ffn['h', n] = (sg * u_).astype(BF)

    def ffn_down(n):
        r = pl.ds(n * 128, min(128, F - n * 128))
        y = jnp.dot(ffn['h', n], wd_v[r, :], preferred_element_type=F32)
        ffn['y'] = y if n == 0 else ffn['y'] + y
        if n == NF - 1:
            rs = _rb(jax.nn.sigmoid(best_m))
            upd_v[...] = jnp.where(row_sel, _rb(_rb(ffn['y']) * rs), 0.0)

    ffn_items = []
    for n in range(NF):
        ffn_items += [functools.partial(ffn_gate, n), functools.partial(ffn_up, n)]
        if n > 0:
            ffn_items.append(functools.partial(ffn_down, n - 1))
    ffn_items.append(functools.partial(ffn_down, NF - 1))

    lane = lax.broadcasted_iota(I32, (B, 128), 1)
    row = lax.broadcasted_iota(I32, (B, 128), 0)
    qi = lane & (B - 1)
    bias_v[0:B] = jnp.where(row > qi, 0.0, -jnp.inf)
    bias_v[B:2 * B] = jnp.where(row <= qi, 0.0, -jnp.inf)

    def lgrp(r):
        return lax.broadcasted_iota(I32, (r, 128), 1) // B

    gm = [jnp.where(lgrp(8) == p, -1, 0).astype(I32) for p in range(G)]

    def bitmask(r, k):
        return ((lgrp(r) >> k) & 1) == 0

    def zrows(n):
        return jnp.zeros((n, 128), I32)

    def stage(X0, X1, k):
        sh = (B // 2) << k
        A = jnp.concatenate([X0, zrows(sh)], axis=0)
        Bm = jnp.concatenate([zrows(sh), X1], axis=0)
        m = bitmask(A.shape[0], k)
        return jnp.where(m, A, Bm), jnp.where(m, Bm, A)

    lrange = [jnp.full((1, 128), 0x7F000000, I32), jnp.zeros((1, 128), I32)]

    def qk_prep(a, g, s):
        qt = qti[a, pl.ds(g * 64, 64), :]
        tiles = []
        for u in range(NU):
            parts = []
            for hp in range(8):
                if hp // G != u:
                    parts.append(zrows(8))
                    continue
                p = (hp - u * G) ^ s
                x = qt[hp * 8:hp * 8 + 8]
                sh = ((p - s) * B) % 128
                if sh:
                    x = pltpu.roll(x, sh, 1)
                parts.append(x & gm[p])
            tiles.append(jnp.concatenate(parts, axis=0))
        return bb(jnp.concatenate(tiles, axis=1)) if NU > 1 else bb(tiles[0])

    def qk_piece(a, g, s, rhs, r0, r1, slot, accs):
        base = a * 128 + s * B - 256
        r0 = max(r0, -base)
        if r0 >= r1:
            return
        kw = bb(ki[g, pl.ds((base + r0) // 2, (r1 - r0) // 2), :])
        Sx = jnp.dot(kw, rhs, preferred_element_type=F32)
        for u in range(NU):
            Sc = Sx[:, u * 128:(u + 1) * 128]
            acc = accs.get((u, s))
            for r in range(r0, r1, 16):
                sr = Sc[r - r0:r - r0 + 16]
                if r < B:
                    sr = sr + bias_v[r:r + 16]
                if r >= 256:
                    sr = sr + bias_v[B + r - 256:B + r - 256 + 16]
                p = jnp.exp2(sr)
                t = p[0:8] + p[8:16]
                acc = t if acc is None else acc + t
                pbuf[slot, u * G + s, r:r + 16] = p.astype(BF)
            accs[(u, s)] = acc

    def pv_prep(a, slot, accs, u):
        idx = {}
        for s in range(G):
            base = a * 128 + s * B - 256
            if base >= 0:
                idx[(s, 0)] = pbi[slot, u * G + s, 0:NR // 2]
            else:
                z = min(-base, NR)
                idx[(s, 0)] = jnp.concatenate(
                    [zrows(z // 2), pbi[slot, u * G + s, z // 2:NR // 2]], axis=0)
        lidx = {(s, 0): jnp.sum(accs[(u, s)], axis=0, keepdims=True) for s in range(G)}
        if CHECK:
            for s in range(G):
                lb = pltpu.bitcast(lidx[(s, 0)], I32)
                lrange[0] = jnp.minimum(lrange[0], lb)
                lrange[1] = jnp.maximum(lrange[1], lb)
        for k in range(LG):
            nidx = {}
            nl = {}
            for sh in range(G >> (k + 1)):
                for c in range(1 << k):
                    Y0, Y1 = stage(idx[(2 * sh, c)], idx[(2 * sh + 1, c)], k)
                    nidx[(sh, c)] = Y0
                    nidx[(sh, c | (1 << k))] = Y1
                    m1 = bitmask(1, k)
                    la, lb = lidx[(2 * sh, c)], lidx[(2 * sh + 1, c)]
                    nl[(sh, c)] = jnp.where(m1, la, lb)
                    nl[(sh, c | (1 << k))] = jnp.where(m1, lb, la)
            idx = nidx
            lidx = nl
        return idx, lidx

    def pv_tile(a, g, u, eta, kt, W, oacc):
        key0 = a * 128 - 256 + kt * 128
        if key0 < 0:
            return
        h = g * 8 + u * G + eta
        vt = bb(vti[key0 // 128, pl.ds(h * 8, 8), :])
        o = jnp.dot(vt, bb(W[(0, eta)][kt * 64:(kt + 1) * 64]), preferred_element_type=F32)
        oacc[(u, eta)] = o if (u, eta) not in oacc else oacc[(u, eta)] + o

    def pv_fin(a, g, u, eta, lidx, oacc):
        h = g * 8 + u * G + eta
        l = lidx[(0, eta)]
        r0 = pltpu.reciprocal(l, approx=True)
        r1 = r0 * (2.0 - l * r0)
        ob = bi((oacc[(u, eta)] * r1).astype(BF))
        for k in range(LG):
            if (eta >> k) & 1:
                d = B << k
                if d == 64:
                    ob = pltpu.roll(ob, 64, 1)
                else:
                    ob = jnp.where(bitmask(8, k), pltpu.roll(ob, 128 - d, 1), pltpu.roll(ob, d, 1))
        ot_v[a, pl.ds(h * 16, 16), :] = bb(ob)

    def out_copy(a):
        r = pl.ds(a * T3 if isinstance(a, int) else pl.multiple_of(a * T3, T3), T3)
        return pltpu.make_async_copy(out_v.at[r], out_hbm.at[r], o_sem.at[0])

    steps = [(a, g) for a in range(NQ) for g in range(4)]
    prev = None
    for n in range(len(steps) + 1):
        qslots = []
        pslots = []
        accs = {}
        if n < len(steps):
            a, g = steps[n]
            rh = {}
            grp = 4 if G == 8 else 2
            for s0 in range(0, G, grp):
                for pi in range(len(CUTS) - 1):
                    qslots.append((list(range(s0, s0 + grp)), CUTS[pi], CUTS[pi + 1]))
        if prev is not None:
            pa, pg, pslot, paccs = prev
            pre = {}
            oacc = {}
            tiles = [(u, kt, e) for u in range(NU) for kt in range(3) for e in range(G)]
            per = 4
            for i in range(0, len(tiles), per):
                pslots.append(tiles[i:i + per])
        for i in range(max(len(qslots), len(pslots))):
            if i < len(qslots):
                ss, r0, r1 = qslots[i]
                for s_ in ss:
                    if s_ not in rh:
                        rh[s_] = qk_prep(a, g, s_)
                    qk_piece(a, g, s_, rh[s_], r0, r1, n % 2, accs)
            if ffn_items and i in FSLOTS and n >= FSTART:
                ffn_items.pop(0)()
            if i < len(pslots):
                for (u, kt, eta) in pslots[i]:
                    if u not in pre:
                        pre[u] = pv_prep(pa, pslot, paccs, u)
                    pv_tile(pa, pg, u, eta, kt, pre[u][0], oacc)
                    if kt == 2:
                        pv_fin(pa, pg, u, eta, pre[u][1], oacc)
        prev = (a, g, n % 2, accs) if n < len(steps) else None
    assert not ffn_items

    def safe_attention():
        rowh = lax.broadcasted_iota(I32, (128, 128), 0) // 16
        kj = lax.broadcasted_iota(I32, (128, 128), 0)
        qi_ = lax.broadcasted_iota(I32, (128, 128), 1)

        def body(t, c):
            a = t // 32
            h = t % 32
            g = h // 8
            qt = qt_v[a, pl.ds(pl.multiple_of(g * 128, 128), 128), :]
            rhs = jnp.where(rowh == h % 8, qt, jnp.zeros_like(qt))
            ss = []
            kbs = []
            for kt in range(3):
                kb = a - 2 + kt
                kbc = jnp.maximum(kb, 0)
                kbs.append(kbc)
                kw = k_v[g, pl.ds(pl.multiple_of(kbc * 128, 128), 128), :]
                sc = jnp.dot(kw, rhs, preferred_element_type=F32)
                d = (a - kb) * 128 + qi_ - kj
                ss.append(jnp.where((kb >= 0) & (d >= 0) & (d < 256), sc, -1e9 * LOG2E))
            m = jnp.max(jnp.maximum(jnp.maximum(ss[0], ss[1]), ss[2]), axis=0, keepdims=True)
            l = None
            o = None
            for kt in range(3):
                p = jnp.exp2(ss[kt] - m)
                lt = jnp.sum(p, axis=0, keepdims=True)
                l = lt if l is None else l + lt
                vt = vt_v[kbs[kt], pl.ds(pl.multiple_of(h * 16, 16), 16), :]
                ot = jnp.dot(vt, p.astype(BF), preferred_element_type=F32)
                o = ot if o is None else o + ot
            ot_v[a, pl.ds(pl.multiple_of(h * 16, 16), 16), :] = (o / l).astype(BF)
            return c

        lax.fori_loop(0, NQ * 32, body, 0)

    if CHECK:
        lo_ok = jnp.min(lrange[0]) >= L_LO
        hi_ok = jnp.max(lrange[1]) <= L_HI
        pl.when(jnp.logical_not(jnp.logical_and(lo_ok, hi_ok)) | FORCE_SAFE)(safe_attention)
    def p3_block(a, par):
        r0 = a * 128 if isinstance(a, int) else pl.multiple_of(a * 128, 128)
        r = pl.ds(r0, 128)
        on_v[par] = ot_v[a].T
        att = jnp.dot(on_v[par], wo_v[...], preferred_element_type=F32)
        if RESP == 1:
            out_v[r, :] = (att + res_v[r, :]).astype(BF)
        else:
            x = x_v[r, :].astype(F32)
            ri = jnp.concatenate([ri_v[r, :]] * 4, axis=1)
            mb = jnp.concatenate([mb_v[r, :]] * 4, axis=1)
            ups = jnp.concatenate([jnp.where(r0 + 16 * t == blk, upd_v[...], 0.0) for t in range(8)], axis=0)
            out_v[r, :] = (att + (x + (x * ri - mb)) + ups).astype(BF)
        out_copy(a).start()

    if P3U == NQ:
        for a in range(NQ):
            p3_block(a, a % 2)
    else:
        def p3_body(i, c):
            for j in range(P3U):
                p3_block(i * P3U + j, j % 2)
            return c

        lax.fori_loop(0, NQ // P3U, p3_body, 0)
    for a in range(NQ):
        out_copy(a).wait()


@jax.jit
def pallas_parallel_sum__sliding_block__moe_arch_mod__prompt_kernel(
    A_x, A_wqkv, A_wo, B_x, B_w_r, B_w_gate, B_w_up, B_w_down,
):
    x = A_x.reshape(S, D)
    anyspec = pl.BlockSpec(memory_space=pltpu.HBM)
    out = pl.pallas_call(
        _kernel,
        out_shape=jax.ShapeDtypeStruct((S, D), BF),
        in_specs=[anyspec, anyspec, anyspec, pl.BlockSpec(memory_space=pltpu.VMEM), anyspec, anyspec, anyspec],
        out_specs=anyspec,
        scratch_shapes=[
            pltpu.VMEM((S, D), BF),
            pltpu.VMEM((D, 3 * D), BF),
            pltpu.VMEM((D, D), BF),
            pltpu.VMEM((F, D), BF),
            pltpu.VMEM((F, D), BF),
            pltpu.VMEM((F, D), BF),
            pltpu.VMEM((S, 128), F32),
            pltpu.VMEM((S, 128), F32),
            pltpu.VMEM((12, 8, 128), F32),
            pltpu.VMEM((S, D), F32),
            pltpu.VMEM((16, D), F32),
            pltpu.VMEM((4, S, 128), BF),
            pltpu.VMEM((NQ, D, 128), BF),
            pltpu.VMEM((NQ, D, 128), BF),
            pltpu.VMEM((2, 8, NR, 128), BF),
            pltpu.VMEM((2 * B, 128), F32),
            pltpu.VMEM((NQ, D, 128), BF),
            pltpu.VMEM((2, 128, D), BF),
            pltpu.VMEM((S, D), BF),
            pltpu.SemaphoreType.DMA((3,)),
            pltpu.SemaphoreType.DMA((7,)),
            pltpu.SemaphoreType.DMA((1,)),
        ],
        compiler_params=pltpu.CompilerParams(vmem_limit_bytes=100 * 2**20),
    )(x, A_wqkv, A_wo, B_w_r, B_w_gate.T, B_w_up.T, B_w_down)
    return out.reshape(1, S, D)
```

```python
import functools
ORDER = [int(c, 16) for c in '012389ab4567']
SPLITDOT = int('0')
P3N = int('1')
RESP = int('3')
SLABS = [int(c) for c in '012']
NF = 11
FSLOTS = [int(c) for c in '0']
FSTART = int('0')
CHECK = int('1')
FORCE_SAFE = bool(int('0'))
L_LO = (127 - 40) << 23
L_HI = (127 + 40) << 23
KE = int('2')
KOFF = int('1')
KSLOT = int('5')
SPLIT0 = int('1')
P3U = int('8')
LOOKAHEAD = int('1')
import jax
import jax.numpy as jnp
import numpy as np
from jax import lax
import jax.experimental.pallas as pl
import jax.experimental.pallas.tpu as pltpu

S = 2048
D = 512
F = 1376
T1 = int('512')
N1 = S // T1
NQ = S // 128
LOG2E = 1.4426950408889634
QSCALE = 0.25 * LOG2E
G = 8
B = 128 // G
NR = 256 + B
LG = 3
NU = 8 // G
OPD = 1
T3 = 128
CUTS = tuple(int(c) for c in '0,112,192,272'.split(','))
PER = int('4')
PO = int('1')
PVFIRST = int('0')
SG = int('0')
BF = jnp.bfloat16
F32 = jnp.float32
I32 = jnp.int32
NT = (((1,), (1,)), ((), ()))
TN = (((0,), (0,)), ((), ()))


def _np_bf16(v):
    u = np.array([v], np.float32).view(np.uint32)
    u = (u + 0x7FFF + ((u >> 16) & 1)) & 0xFFFF0000
    return float(u.astype(np.uint32).view(np.float32)[0])


EPS_B = _np_bf16(1e-5)


def bi(x):
    return pltpu.bitcast(x, I32)


def bb(x):
    return pltpu.bitcast(x, BF)


def _rb(x):
    return x.astype(BF).astype(F32)


def _kernel(x_hbm, wqkv_hbm, wo_hbm, wr_ref, wg_hbm, wu_hbm, wd_hbm, out_hbm,
            x_v, wqkv_v, wo_v, wg_v, wu_v, wd_v,
            mb_v, ri_v, cs_v, res_v, upd_v, k_v, qt_v, vt_v, pbuf, bias_v, ot_v, on_v, out_v,
            x_sem, w_sem, o_sem):
    XCH = [(0, 256), (256, 256), (T1, T1), (2 * T1, S - 2 * T1)] if SPLIT0 else [(0, T1), (T1, T1), (2 * T1, S - 2 * T1)]

    def x_copy(j):
        r = pl.ds(*XCH[j])
        return pltpu.make_async_copy(x_hbm.at[r], x_v.at[r], x_sem.at[j])

    def wq_copy(j):
        c = pl.ds(j * D, D)
        return pltpu.make_async_copy(wqkv_hbm.at[:, c], wqkv_v.at[:, c], w_sem.at[j])

    wo_copy = pltpu.make_async_copy(wo_hbm, wo_v, w_sem.at[3])
    ffn_copies = [
        pltpu.make_async_copy(wg_hbm, wg_v, w_sem.at[4]),
        pltpu.make_async_copy(wu_hbm, wu_v, w_sem.at[5]),
        pltpu.make_async_copy(wd_hbm, wd_v, w_sem.at[6]),
    ]
    x_copy(0).start()
    wq_copy(0).start()
    if SPLIT0:
        x_copy(1).start()
    wq_copy(1).start()
    wq_copy(2).start()
    x_copy(2 if SPLIT0 else 1).start()

    wr = wr_ref[...].astype(F32).reshape(1, D)
    ki = k_v.bitcast(I32)
    qti = qt_v.bitcast(I32)
    pbi = pbuf.bitcast(I32)
    vti = vt_v.bitcast(I32)

    swr = jnp.sum(wr, axis=1, keepdims=True)

    def row_stats(x):
        mean = jnp.mean(x, axis=1, keepdims=True)
        c = x - mean
        var = jnp.mean(c * c, axis=1, keepdims=True)
        mb = _rb(mean)
        sd = _rb(jnp.sqrt(_rb(_rb(var) + EPS_B)))
        return mb, sd

    def stats(r0, nr, best_m, best_i):
        r = pl.ds(r0, nr)
        x = x_v[r, :].astype(F32)
        mb, sd = row_stats(x)
        ri = 1.0 / sd
        mb_v[r, :] = jnp.broadcast_to(mb * ri, (nr, 128))
        ri_v[r, :] = jnp.broadcast_to(ri, (nr, 128))
        rr = _rb((jnp.sum(x * wr, axis=1, keepdims=True) - mb * swr) * ri)
        m = jnp.max(rr, axis=0, keepdims=True)
        rows = lax.broadcasted_iota(I32, (nr, 1), 0) + r0
        idx = jnp.min(jnp.where(rr == m, rows, S), axis=0, keepdims=True)
        better = m > best_m
        return jnp.where(better, m, best_m), jnp.where(better, idx, best_i)

    def colsum(ns):
        for n in ns:
            cs_v[n] = jnp.dot(jnp.ones((16, D), BF), wqkv_v[:, n * 128:(n + 1) * 128],
                              preferred_element_type=F32)[0:8]

    def project(b0, nb, ns):
        r = pl.ds(b0 * 128 if isinstance(b0, int) else pl.multiple_of(b0 * 128, 128), nb * 128)
        accs = {n: jnp.dot(x_v[r, :], wqkv_v[:, n * 128:(n + 1) * 128], preferred_element_type=F32) for n in ns}
        mb = mb_v[r, :]
        ri = ri_v[r, :]
        for n in ns:
            cs = jnp.broadcast_to(cs_v[n, 0:1, :], (nb * 128, 128))
            y = accs[n] * ri - mb * cs
            if n < 4:
                y = y * QSCALE
                for j in range(nb):
                    qt_v[b0 + j, n * 128:(n + 1) * 128, :] = y[j * 128:(j + 1) * 128].T.astype(BF)
            elif n < 8:
                k_v[n - 4, r, :] = y.astype(BF)
            else:
                for j in range(nb):
                    vt_v[b0 + j, (n - 8) * 128:(n - 7) * 128, :] = y[j * 128:(j + 1) * 128].T.astype(BF)

    QN, KN, VN = range(0, 4), range(4, 8), range(8, 12)
    carry = (jnp.full((1, 1), -jnp.inf, F32), jnp.full((1, 1), S - 1, I32))
    if SPLIT0:
        x_copy(0).wait()
        carry = stats(0, 256, *carry)
        wq_copy(0).wait()
        x_copy(3).start()
        wo_copy.start()
        colsum(QN)
        project(0, 2, QN)
        x_copy(1).wait()
        wq_copy(1).wait()
        colsum(KN)
        carry = stats(256, 256, *carry)
        project(0, 2, KN)
        project(2, 2, list(QN) + list(KN))
        wq_copy(2).wait()
        x_copy(2).wait()
        colsum(VN)
        project(0, 4, VN)
    else:
        x_copy(0).wait()
        carry = stats(0, T1, *carry)
        for t, ns in enumerate((QN, KN, VN)):
            wq_copy(t).wait()
            if t == 0:
                x_copy(2).start()
                wo_copy.start()
            if t == 2:
                x_copy(1).wait()
            colsum(ns)
            project(0, 4, ns)
    carry = stats(T1, T1, *carry)

    def p1_body(i, carry):
        @pl.when(i == 1)
        def _():
            x_copy(len(XCH) - 1).wait()
            for c in ffn_copies:
                c.start()

        @pl.when(i == N1 - 1)
        def _():
            for c in ffn_copies:
                c.wait()
            wo_copy.wait()
        project(i * 4, 4, ORDER)
        return stats(pl.multiple_of(jnp.minimum(i + 1, N1 - 1) * T1, T1), T1, *carry)

    best_m, best_i = lax.fori_loop(1, N1, p1_body, carry)

    idx = jnp.clip(jnp.max(best_i), 0, S - 1)
    blk = pl.multiple_of((idx // 16) * 16, 16)
    row_sel = lax.broadcasted_iota(I32, (16, 1), 0) == (idx - blk)
    xr = x_v[pl.ds(blk, 16), :].astype(F32)
    mbr, sdr = row_stats(xr)
    xs = jnp.where(row_sel, _rb(xr - mbr) / sdr, 0.0).astype(BF)
    ffn = {}

    def ffn_gate(n):
        r = pl.ds(n * 128, min(128, F - n * 128))
        ffn['g', n] = _rb(lax.dot_general(xs, wg_v[r, :], NT, preferred_element_type=F32))

    def ffn_up(n):
        r = pl.ds(n * 128, min(128, F - n * 128))
        u_ = _rb(lax.dot_general(xs, wu_v[r, :], NT, preferred_element_type=F32))
        g_ = ffn['g', n]
        sg = _rb(g_ * _rb(jax.nn.sigmoid(g_)))
        ffn['h', n] = (sg * u_).astype(BF)

    def ffn_down(n):
        r = pl.ds(n * 128, min(128, F - n * 128))
        y = jnp.dot(ffn['h', n], wd_v[r, :], preferred_element_type=F32)
        ffn['y'] = y if n == 0 else ffn['y'] + y
        if n == NF - 1:
            rs = _rb(jax.nn.sigmoid(best_m))
            upd_v[...] = jnp.where(row_sel, _rb(_rb(ffn['y']) * rs), 0.0)

    ffn_items = []
    for n in range(NF):
        ffn_items += [functools.partial(ffn_gate, n), functools.partial(ffn_up, n)]
        if n > 0:
            ffn_items.append(functools.partial(ffn_down, n - 1))
    ffn_items.append(functools.partial(ffn_down, NF - 1))

    lane = lax.broadcasted_iota(I32, (B, 128), 1)
    row = lax.broadcasted_iota(I32, (B, 128), 0)
    qi = lane & (B - 1)
    bias_v[0:B] = jnp.where(row > qi, 0.0, -jnp.inf)
    bias_v[B:2 * B] = jnp.where(row <= qi, 0.0, -jnp.inf)

    def lgrp(r):
        return lax.broadcasted_iota(I32, (r, 128), 1) // B

    gm = [jnp.where(lgrp(8) == p, -1, 0).astype(I32) for p in range(G)]

    def bitmask(r, k):
        return ((lgrp(r) >> k) & 1) == 0

    def zrows(n):
        return jnp.zeros((n, 128), I32)

    def stage(X0, X1, k):
        sh = (B // 2) << k
        A = jnp.concatenate([X0, zrows(sh)], axis=0)
        Bm = jnp.concatenate([zrows(sh), X1], axis=0)
        m = bitmask(A.shape[0], k)
        return jnp.where(m, A, Bm), jnp.where(m, Bm, A)

    lrange = [jnp.full((1, 128), 0x7F000000, I32), jnp.zeros((1, 128), I32)]

    def qk_prep(a, g, s):
        qt = qti[a, pl.ds(g * 64, 64), :]
        tiles = []
        for u in range(NU):
            parts = []
            for hp in range(8):
                if hp // G != u:
                    parts.append(zrows(8))
                    continue
                p = (hp - u * G) ^ s
                x = qt[hp * 8:hp * 8 + 8]
                sh = ((p - s) * B) % 128
                if sh:
                    x = pltpu.roll(x, sh, 1)
                parts.append(x & gm[p])
            tiles.append(jnp.concatenate(parts, axis=0))
        return bb(jnp.concatenate(tiles, axis=1)) if NU > 1 else bb(tiles[0])

    def qk_piece(a, g, s, rhs, r0, r1, slot, accs):
        base = a * 128 + s * B - 256
        r0 = max(r0, -base)
        if r0 >= r1:
            return
        kw = bb(ki[g, pl.ds((base + r0) // 2, (r1 - r0) // 2), :])
        Sx = jnp.dot(kw, rhs, preferred_element_type=F32)
        for u in range(NU):
            Sc = Sx[:, u * 128:(u + 1) * 128]
            acc = accs.get((u, s))
            for r in range(r0, r1, 16):
                sr = Sc[r - r0:r - r0 + 16]
                if r < B:
                    sr = sr + bias_v[r:r + 16]
                if r >= 256:
                    sr = sr + bias_v[B + r - 256:B + r - 256 + 16]
                p = jnp.exp2(sr)
                t = p[0:8] + p[8:16]
                acc = t if acc is None else acc + t
                pbuf[slot, u * G + s, r:r + 16] = p.astype(BF)
            accs[(u, s)] = acc

    def pv_prep(a, slot, accs, u):
        idx = {}
        for s in range(G):
            base = a * 128 + s * B - 256
            if base >= 0:
                idx[(s, 0)] = pbi[slot, u * G + s, 0:NR // 2]
            else:
                z = min(-base, NR)
                idx[(s, 0)] = jnp.concatenate(
                    [zrows(z // 2), pbi[slot, u * G + s, z // 2:NR // 2]], axis=0)
        lidx = {(s, 0): jnp.sum(accs[(u, s)], axis=0, keepdims=True) for s in range(G)}
        if CHECK:
            for s in range(G):
                lb = pltpu.bitcast(lidx[(s, 0)], I32)
                lrange[0] = jnp.minimum(lrange[0], lb)
                lrange[1] = jnp.maximum(lrange[1], lb)
        for k in range(LG):
            nidx = {}
            nl = {}
            for sh in range(G >> (k + 1)):
                for c in range(1 << k):
                    Y0, Y1 = stage(idx[(2 * sh, c)], idx[(2 * sh + 1, c)], k)
                    nidx[(sh, c)] = Y0
                    nidx[(sh, c | (1 << k))] = Y1
                    m1 = bitmask(1, k)
                    la, lb = lidx[(2 * sh, c)], lidx[(2 * sh + 1, c)]
                    nl[(sh, c)] = jnp.where(m1, la, lb)
                    nl[(sh, c | (1 << k))] = jnp.where(m1, lb, la)
            idx = nidx
            lidx = nl
        return idx, lidx

    def pv_tile(a, g, u, eta, kt, W, oacc):
        key0 = a * 128 - 256 + kt * 128
        if key0 < 0:
            return
        h = g * 8 + u * G + eta
        vt = bb(vti[key0 // 128, pl.ds(h * 8, 8), :])
        o = jnp.dot(vt, bb(W[(0, eta)][kt * 64:(kt + 1) * 64]), preferred_element_type=F32)
        oacc[(u, eta)] = o if (u, eta) not in oacc else oacc[(u, eta)] + o

    def pv_fin(a, g, u, eta, lidx, oacc):
        h = g * 8 + u * G + eta
        l = lidx[(0, eta)]
        r0 = pltpu.reciprocal(l, approx=True)
        r1 = r0 * (2.0 - l * r0)
        ob = bi((oacc[(u, eta)] * r1).astype(BF))
        for k in range(LG):
            if (eta >> k) & 1:
                d = B << k
                if d == 64:
                    ob = pltpu.roll(ob, 64, 1)
                else:
                    ob = jnp.where(bitmask(8, k), pltpu.roll(ob, 128 - d, 1), pltpu.roll(ob, d, 1))
        ot_v[a, pl.ds(h * 16, 16), :] = bb(ob)

    def out_copy(a):
        r = pl.ds(a * T3 if isinstance(a, int) else pl.multiple_of(a * T3, T3), T3)
        return pltpu.make_async_copy(out_v.at[r], out_hbm.at[r], o_sem.at[0])

    def p3_block(a, par):
        r0 = a * 128 if isinstance(a, int) else pl.multiple_of(a * 128, 128)
        r = pl.ds(r0, 128)
        on_v[par] = ot_v[a].T
        att = jnp.dot(on_v[par], wo_v[...], preferred_element_type=F32)
        if RESP == 1:
            out_v[r, :] = (att + res_v[r, :]).astype(BF)
        else:
            x = x_v[r, :].astype(F32)
            ri = jnp.concatenate([ri_v[r, :]] * 4, axis=1)
            mb = jnp.concatenate([mb_v[r, :]] * 4, axis=1)
            ups = jnp.concatenate([jnp.where(r0 + 16 * t == blk, upd_v[...], 0.0) for t in range(8)], axis=0)
            out_v[r, :] = (att + (x + (x * ri - mb)) + ups).astype(BF)
        out_copy(a).start()

    steps = [(a, g) for a in range(NQ) for g in range(4)]
    early = list(range(KE))
    prev = None
    for n in range(len(steps) + 1):
        qslots = []
        pslots = []
        accs = {}
        if n < len(steps):
            a, g = steps[n]
            rh = {}
            sgs = [[0, 1, 2, 3], [4, 5, 6, 7]] if SG == 0 else [[0, 2, 4, 6], [1, 3, 5, 7]]
            for ss in sgs:
                for pi in range(len(CUTS) - 1):
                    qslots.append((ss, CUTS[pi], CUTS[pi + 1]))
        if prev is not None:
            pa, pg, pslot, paccs = prev
            pre = {}
            oacc = {}
            if PO == 0:
                tiles = [(0, kt, e) for kt in range(3) for e in range(G)]
            elif PO == 1:
                tiles = [(0, kt, e) for e0 in (0, 4) for kt in range(3) for e in range(e0, e0 + 4)]
            elif PO == 2:
                tiles = [(0, kt, e) for kt in range(3) for e in (0, 2, 4, 6, 1, 3, 5, 7)]
            elif PO == 3:
                tiles = [(0, kt, e) for kt in (1, 0, 2) for e in range(G)]
            for i in range(0, len(tiles), PER):
                pslots.append(tiles[i:i + PER])
        done = {}

        def do_q(i):
            if i < len(qslots):
                ss, r0, r1 = qslots[i]
                for s_ in ss:
                    if s_ not in rh:
                        rh[s_] = qk_prep(a, g, s_)
                    qk_piece(a, g, s_, rh[s_], r0, r1, n % 2, accs)

        def do_p(i):
            if i < len(pslots):
                for (u, kt, eta) in pslots[i]:
                    if u not in pre:
                        pre[u] = pv_prep(pa, pslot, paccs, u)
                    pv_tile(pa, pg, u, eta, kt, pre[u][0], oacc)
                    done[eta] = done.get(eta, 0) + 1
                    if done[eta] == 3:
                        pv_fin(pa, pg, u, eta, pre[u][1], oacc)

        for i in range(max(len(qslots), len(pslots))):
            if PVFIRST:
                do_p(i)
                do_q(i)
            else:
                do_q(i)
            if ffn_items and i in FSLOTS and n >= FSTART:
                ffn_items.pop(0)()
            if not PVFIRST:
                do_p(i)
            if early and n >= len(steps) - KE + KOFF and i == KSLOT:
                a_ = early.pop(0)
                p3_block(a_, a_ % 2)
        prev = (a, g, n % 2, accs) if n < len(steps) else None
    assert not ffn_items
    for a_ in early:
        p3_block(a_, a_ % 2)

    def safe_attention():
        rowh = lax.broadcasted_iota(I32, (128, 128), 0) // 16
        kj = lax.broadcasted_iota(I32, (128, 128), 0)
        qi_ = lax.broadcasted_iota(I32, (128, 128), 1)

        def body(t, c):
            a = t // 32
            h = t % 32
            g = h // 8
            qt = qt_v[a, pl.ds(pl.multiple_of(g * 128, 128), 128), :]
            rhs = jnp.where(rowh == h % 8, qt, jnp.zeros_like(qt))
            ss = []
            kbs = []
            for kt in range(3):
                kb = a - 2 + kt
                kbc = jnp.maximum(kb, 0)
                kbs.append(kbc)
                kw = k_v[g, pl.ds(pl.multiple_of(kbc * 128, 128), 128), :]
                sc = jnp.dot(kw, rhs, preferred_element_type=F32)
                d = (a - kb) * 128 + qi_ - kj
                ss.append(jnp.where((kb >= 0) & (d >= 0) & (d < 256), sc, -1e9 * LOG2E))
            m = jnp.max(jnp.maximum(jnp.maximum(ss[0], ss[1]), ss[2]), axis=0, keepdims=True)
            l = None
            o = None
            for kt in range(3):
                p = jnp.exp2(ss[kt] - m)
                lt = jnp.sum(p, axis=0, keepdims=True)
                l = lt if l is None else l + lt
                vt = vt_v[kbs[kt], pl.ds(pl.multiple_of(h * 16, 16), 16), :]
                ot = jnp.dot(vt, p.astype(BF), preferred_element_type=F32)
                o = ot if o is None else o + ot
            ot_v[a, pl.ds(pl.multiple_of(h * 16, 16), 16), :] = (o / l).astype(BF)
            return c

        lax.fori_loop(0, NQ * 32, body, 0)
        for a_ in range(KE):
            out_copy(a_).wait()

        def redo(a_, c):
            p3_block(a_, 0)
            return c

        lax.fori_loop(0, KE, redo, 0)

    if CHECK:
        lo_ok = jnp.min(lrange[0]) >= L_LO
        hi_ok = jnp.max(lrange[1]) <= L_HI
        pl.when(jnp.logical_not(jnp.logical_and(lo_ok, hi_ok)) | FORCE_SAFE)(safe_attention)
    n3 = (NQ - KE) // 2

    def p3_body(i, c):
        for j in range(n3):
            p3_block(KE + i * n3 + j, j % 2)
        return c

    lax.fori_loop(0, 2, p3_body, 0)
    for a in range(NQ):
        out_copy(a).wait()


@jax.jit
def pallas_parallel_sum__sliding_block__moe_arch_mod__prompt_kernel(
    A_x, A_wqkv, A_wo, B_x, B_w_r, B_w_gate, B_w_up, B_w_down,
):
    x = A_x.reshape(S, D)
    anyspec = pl.BlockSpec(memory_space=pltpu.HBM)
    out = pl.pallas_call(
        _kernel,
        out_shape=jax.ShapeDtypeStruct((S, D), BF),
        in_specs=[anyspec, anyspec, anyspec, pl.BlockSpec(memory_space=pltpu.VMEM), anyspec, anyspec, anyspec],
        out_specs=anyspec,
        scratch_shapes=[
            pltpu.VMEM((S, D), BF),
            pltpu.VMEM((D, 3 * D), BF),
            pltpu.VMEM((D, D), BF),
            pltpu.VMEM((F, D), BF),
            pltpu.VMEM((F, D), BF),
            pltpu.VMEM((F, D), BF),
            pltpu.VMEM((S, 128), F32),
            pltpu.VMEM((S, 128), F32),
            pltpu.VMEM((12, 8, 128), F32),
            pltpu.VMEM((S, D), F32),
            pltpu.VMEM((16, D), F32),
            pltpu.VMEM((4, S, 128), BF),
            pltpu.VMEM((NQ, D, 128), BF),
            pltpu.VMEM((NQ, D, 128), BF),
            pltpu.VMEM((2, 8, NR, 128), BF),
            pltpu.VMEM((2 * B, 128), F32),
            pltpu.VMEM((NQ, D, 128), BF),
            pltpu.VMEM((2, 128, D), BF),
            pltpu.VMEM((S, D), BF),
            pltpu.SemaphoreType.DMA((4,)),
            pltpu.SemaphoreType.DMA((7,)),
            pltpu.SemaphoreType.DMA((1,)),
        ],
        compiler_params=pltpu.CompilerParams(vmem_limit_bytes=100 * 2**20),
    )(x, A_wqkv, A_wo, B_w_r, B_w_gate.T, B_w_up.T, B_w_down)
    return out.reshape(1, S, D)
```

```python
import functools

import jax
import jax.numpy as jnp
import numpy as np
from jax import lax
import jax.experimental.pallas as pl
import jax.experimental.pallas.tpu as pltpu

S = 2048
D = 512
F = 1376
NF = 11
T1 = 512
N1 = S // T1
NQ = S // 128
LOG2E = 1.4426950408889634
QSCALE = 0.25 * LOG2E
G = 8
B = 128 // G
NR = 256 + B
LG = 3
CUTS = (0, 112, 192, NR)
ORDER = (0, 1, 2, 3, 8, 9, 10, 11, 4, 5, 6, 7)
KE = 2
L_LO = (127 - 40) << 23
L_HI = (127 + 40) << 23
BF = jnp.bfloat16
F32 = jnp.float32
I32 = jnp.int32
NT = (((1,), (1,)), ((), ()))


def _np_bf16(v):
    u = np.array([v], np.float32).view(np.uint32)
    u = (u + 0x7FFF + ((u >> 16) & 1)) & 0xFFFF0000
    return float(u.astype(np.uint32).view(np.float32)[0])


EPS_B = _np_bf16(1e-5)


def bi(x):
    return pltpu.bitcast(x, I32)


def bb(x):
    return pltpu.bitcast(x, BF)


def _rb(x):
    return x.astype(BF).astype(F32)


def _kernel(x_hbm, wqkv_hbm, wo_hbm, wr_ref, wg_hbm, wu_hbm, wd_hbm, out_hbm,
            x_v, wqkv_v, wo_v, wg_v, wu_v, wd_v,
            mb_v, ri_v, cs_v, upd_v, k_v, qt_v, vt_v, pbuf, bias_v, ot_v, on_v, out_v,
            x_sem, w_sem, o_sem):
    XCH = [(0, 256), (256, 256), (T1, T1), (2 * T1, S - 2 * T1)]

    def x_copy(j):
        r = pl.ds(*XCH[j])
        return pltpu.make_async_copy(x_hbm.at[r], x_v.at[r], x_sem.at[j])

    def wq_copy(j):
        c = pl.ds(j * D, D)
        return pltpu.make_async_copy(wqkv_hbm.at[:, c], wqkv_v.at[:, c], w_sem.at[j])

    wo_copy = pltpu.make_async_copy(wo_hbm, wo_v, w_sem.at[3])
    ffn_copies = [
        pltpu.make_async_copy(wg_hbm, wg_v, w_sem.at[4]),
        pltpu.make_async_copy(wu_hbm, wu_v, w_sem.at[5]),
        pltpu.make_async_copy(wd_hbm, wd_v, w_sem.at[6]),
    ]
    x_copy(0).start()
    wq_copy(0).start()
    x_copy(1).start()
    wq_copy(1).start()
    wq_copy(2).start()
    x_copy(2).start()

    wr = wr_ref[...].astype(F32).reshape(1, D)
    ki = k_v.bitcast(I32)
    qti = qt_v.bitcast(I32)
    pbi = pbuf.bitcast(I32)
    vti = vt_v.bitcast(I32)

    swr = jnp.sum(wr, axis=1, keepdims=True)

    def row_stats(x):
        mean = jnp.mean(x, axis=1, keepdims=True)
        c = x - mean
        var = jnp.mean(c * c, axis=1, keepdims=True)
        mb = _rb(mean)
        sd = _rb(jnp.sqrt(_rb(_rb(var) + EPS_B)))
        return mb, sd

    def stats(r0, nr, best_m, best_i):
        r = pl.ds(r0, nr)
        x = x_v[r, :].astype(F32)
        mb, sd = row_stats(x)
        ri = 1.0 / sd
        mb_v[r, :] = jnp.broadcast_to(mb * ri, (nr, 128))
        ri_v[r, :] = jnp.broadcast_to(ri, (nr, 128))
        rr = _rb((jnp.sum(x * wr, axis=1, keepdims=True) - mb * swr) * ri)
        m = jnp.max(rr, axis=0, keepdims=True)
        rows = lax.broadcasted_iota(I32, (nr, 1), 0) + r0
        idx = jnp.min(jnp.where(rr == m, rows, S), axis=0, keepdims=True)
        better = m > best_m
        return jnp.where(better, m, best_m), jnp.where(better, idx, best_i)

    def colsum(ns):
        for n in ns:
            cs_v[n] = jnp.dot(jnp.ones((16, D), BF), wqkv_v[:, n * 128:(n + 1) * 128],
                              preferred_element_type=F32)[0:8]

    def project(b0, nb, ns):
        r = pl.ds(b0 * 128 if isinstance(b0, int) else pl.multiple_of(b0 * 128, 128), nb * 128)
        accs = {n: jnp.dot(x_v[r, :], wqkv_v[:, n * 128:(n + 1) * 128], preferred_element_type=F32) for n in ns}
        mb = mb_v[r, :]
        ri = ri_v[r, :]
        for n in ns:
            cs = jnp.broadcast_to(cs_v[n, 0:1, :], (nb * 128, 128))
            y = accs[n] * ri - mb * cs
            if n < 4:
                y = y * QSCALE
                for j in range(nb):
                    qt_v[b0 + j, n * 128:(n + 1) * 128, :] = y[j * 128:(j + 1) * 128].T.astype(BF)
            elif n < 8:
                k_v[n - 4, r, :] = y.astype(BF)
            else:
                for j in range(nb):
                    vt_v[b0 + j, (n - 8) * 128:(n - 7) * 128, :] = y[j * 128:(j + 1) * 128].T.astype(BF)

    QN, KN, VN = range(0, 4), range(4, 8), range(8, 12)
    carry = (jnp.full((1, 1), -jnp.inf, F32), jnp.full((1, 1), S - 1, I32))
    x_copy(0).wait()
    carry = stats(0, 256, *carry)
    wq_copy(0).wait()
    x_copy(3).start()
    wo_copy.start()
    colsum(QN)
    project(0, 2, QN)
    x_copy(1).wait()
    wq_copy(1).wait()
    colsum(KN)
    carry = stats(256, 256, *carry)
    project(0, 2, KN)
    project(2, 2, list(QN) + list(KN))
    wq_copy(2).wait()
    x_copy(2).wait()
    colsum(VN)
    project(0, 4, VN)
    carry = stats(T1, T1, *carry)

    def p1_body(i, carry):
        @pl.when(i == 1)
        def _():
            x_copy(3).wait()
            for c in ffn_copies:
                c.start()

        @pl.when(i == N1 - 1)
        def _():
            for c in ffn_copies:
                c.wait()
            wo_copy.wait()

        project(i * 4, 4, ORDER)
        return stats(pl.multiple_of(jnp.minimum(i + 1, N1 - 1) * T1, T1), T1, *carry)

    best_m, best_i = lax.fori_loop(1, N1, p1_body, carry)

    idx = jnp.clip(jnp.max(best_i), 0, S - 1)
    blk = pl.multiple_of((idx // 16) * 16, 16)
    row_sel = lax.broadcasted_iota(I32, (16, 1), 0) == (idx - blk)
    xr = x_v[pl.ds(blk, 16), :].astype(F32)
    mbr, sdr = row_stats(xr)
    xs = jnp.where(row_sel, _rb(xr - mbr) / sdr, 0.0).astype(BF)
    ffn = {}

    def ffn_gate(n):
        r = pl.ds(n * 128, min(128, F - n * 128))
        ffn['g', n] = _rb(lax.dot_general(xs, wg_v[r, :], NT, preferred_element_type=F32))

    def ffn_up(n):
        r = pl.ds(n * 128, min(128, F - n * 128))
        u_ = _rb(lax.dot_general(xs, wu_v[r, :], NT, preferred_element_type=F32))
        g_ = ffn['g', n]
        sg = _rb(g_ * _rb(jax.nn.sigmoid(g_)))
        ffn['h', n] = (sg * u_).astype(BF)

    def ffn_down(n):
        r = pl.ds(n * 128, min(128, F - n * 128))
        y = jnp.dot(ffn['h', n], wd_v[r, :], preferred_element_type=F32)
        ffn['y'] = y if n == 0 else ffn['y'] + y
        if n == NF - 1:
            rs = _rb(jax.nn.sigmoid(best_m))
            upd_v[...] = jnp.where(row_sel, _rb(_rb(ffn['y']) * rs), 0.0)

    ffn_items = []
    for n in range(NF):
        ffn_items += [functools.partial(ffn_gate, n), functools.partial(ffn_up, n)]
        if n > 0:
            ffn_items.append(functools.partial(ffn_down, n - 1))
    ffn_items.append(functools.partial(ffn_down, NF - 1))

    lane = lax.broadcasted_iota(I32, (B, 128), 1)
    row = lax.broadcasted_iota(I32, (B, 128), 0)
    qi = lane & (B - 1)
    bias_v[0:B] = jnp.where(row > qi, 0.0, -jnp.inf)
    bias_v[B:2 * B] = jnp.where(row <= qi, 0.0, -jnp.inf)

    def lgrp(r):
        return lax.broadcasted_iota(I32, (r, 128), 1) // B

    gm = [jnp.where(lgrp(8) == p, -1, 0).astype(I32) for p in range(G)]

    def bitmask(r, k):
        return ((lgrp(r) >> k) & 1) == 0

    def zrows(n):
        return jnp.zeros((n, 128), I32)

    def stage(X0, X1, k):
        sh = (B // 2) << k
        A = jnp.concatenate([X0, zrows(sh)], axis=0)
        Bm = jnp.concatenate([zrows(sh), X1], axis=0)
        m = bitmask(A.shape[0], k)
        return jnp.where(m, A, Bm), jnp.where(m, Bm, A)

    lrange = [jnp.full((1, 128), 0x7F000000, I32), jnp.zeros((1, 128), I32)]

    def qk_prep(a, g, s):
        qt = qti[a, pl.ds(g * 64, 64), :]
        parts = []
        for hp in range(8):
            p = hp ^ s
            x = qt[hp * 8:hp * 8 + 8]
            sh = ((p - s) * B) % 128
            if sh:
                x = pltpu.roll(x, sh, 1)
            parts.append(x & gm[p])
        return bb(jnp.concatenate(parts, axis=0))

    def qk_piece(a, g, s, rhs, r0, r1, slot, accs):
        base = a * 128 + s * B - 256
        r0 = max(r0, -base)
        if r0 >= r1:
            return
        kw = bb(ki[g, pl.ds((base + r0) // 2, (r1 - r0) // 2), :])
        sc = jnp.dot(kw, rhs, preferred_element_type=F32)
        acc = accs.get(s)
        for r in range(r0, r1, 16):
            sr = sc[r - r0:r - r0 + 16]
            if r < B:
                sr = sr + bias_v[r:r + 16]
            if r >= 256:
                sr = sr + bias_v[B + r - 256:B + r - 256 + 16]
            p = jnp.exp2(sr)
            t = p[0:8] + p[8:16]
            acc = t if acc is None else acc + t
            pbuf[slot, s, r:r + 16] = p.astype(BF)
        accs[s] = acc

    def pv_prep(a, slot, accs):
        idx = {}
        for s in range(G):
            base = a * 128 + s * B - 256
            if base >= 0:
                idx[(s, 0)] = pbi[slot, s, 0:NR // 2]
            else:
                z = min(-base, NR)
                idx[(s, 0)] = jnp.concatenate(
                    [zrows(z // 2), pbi[slot, s, z // 2:NR // 2]], axis=0)
        lidx = {(s, 0): jnp.sum(accs[s], axis=0, keepdims=True) for s in range(G)}
        for s in range(G):
            lb = pltpu.bitcast(lidx[(s, 0)], I32)
            lrange[0] = jnp.minimum(lrange[0], lb)
            lrange[1] = jnp.maximum(lrange[1], lb)
        for k in range(LG):
            nidx = {}
            nl = {}
            for sh in range(G >> (k + 1)):
                for c in range(1 << k):
                    Y0, Y1 = stage(idx[(2 * sh, c)], idx[(2 * sh + 1, c)], k)
                    nidx[(sh, c)] = Y0
                    nidx[(sh, c | (1 << k))] = Y1
                    m1 = bitmask(1, k)
                    la, lb = lidx[(2 * sh, c)], lidx[(2 * sh + 1, c)]
                    nl[(sh, c)] = jnp.where(m1, la, lb)
                    nl[(sh, c | (1 << k))] = jnp.where(m1, lb, la)
            idx = nidx
            lidx = nl
        return idx, lidx

    def pv_tile(a, g, eta, kt, W, oacc):
        key0 = a * 128 - 256 + kt * 128
        if key0 < 0:
            return
        h = g * 8 + eta
        vt = bb(vti[key0 // 128, pl.ds(h * 8, 8), :])
        o = jnp.dot(vt, bb(W[(0, eta)][kt * 64:(kt + 1) * 64]), preferred_element_type=F32)
        oacc[eta] = o if eta not in oacc else oacc[eta] + o

    def pv_fin(a, g, eta, lidx, oacc):
        h = g * 8 + eta
        l = lidx[(0, eta)]
        r0 = pltpu.reciprocal(l, approx=True)
        r1 = r0 * (2.0 - l * r0)
        ob = bi((oacc[eta] * r1).astype(BF))
        for k in range(LG):
            if (eta >> k) & 1:
                d = B << k
                if d == 64:
                    ob = pltpu.roll(ob, 64, 1)
                else:
                    ob = jnp.where(bitmask(8, k), pltpu.roll(ob, 128 - d, 1), pltpu.roll(ob, d, 1))
        ot_v[a, pl.ds(h * 16, 16), :] = bb(ob)

    def out_copy(a):
        r = pl.ds(a * 128 if isinstance(a, int) else pl.multiple_of(a * 128, 128), 128)
        return pltpu.make_async_copy(out_v.at[r], out_hbm.at[r], o_sem.at[0])

    def p3_block(a, par):
        r0 = a * 128 if isinstance(a, int) else pl.multiple_of(a * 128, 128)
        r = pl.ds(r0, 128)
        on_v[par] = ot_v[a].T
        att = jnp.dot(on_v[par], wo_v[...], preferred_element_type=F32)
        x = x_v[r, :].astype(F32)
        ri = jnp.concatenate([ri_v[r, :]] * 4, axis=1)
        mb = jnp.concatenate([mb_v[r, :]] * 4, axis=1)
        ups = jnp.concatenate([jnp.where(r0 + 16 * t == blk, upd_v[...], 0.0) for t in range(8)], axis=0)
        out_v[r, :] = (att + (x + (x * ri - mb)) + ups).astype(BF)
        out_copy(a).start()

    steps = [(a, g) for a in range(NQ) for g in range(4)]
    early = list(range(KE))
    prev = None
    for n in range(len(steps) + 1):
        qslots = []
        pslots = []
        accs = {}
        rh = {}
        pre = []
        oacc = {}
        done = {}
        if n < len(steps):
            a, g = steps[n]
            for ss in ([0, 1, 2, 3], [4, 5, 6, 7]):
                for pi in range(len(CUTS) - 1):
                    qslots.append((ss, CUTS[pi], CUTS[pi + 1]))
        if prev is not None:
            pa, pg, pslot, paccs = prev
            tiles = [(kt, e) for e0 in (0, 4) for kt in range(3) for e in range(e0, e0 + 4)]
            pslots = [tiles[i:i + 4] for i in range(0, len(tiles), 4)]
        for i in range(max(len(qslots), len(pslots))):
            if i < len(qslots):
                ss, r0, r1 = qslots[i]
                for s_ in ss:
                    if s_ not in rh:
                        rh[s_] = qk_prep(a, g, s_)
                    qk_piece(a, g, s_, rh[s_], r0, r1, n % 2, accs)
            if ffn_items and i == 0:
                ffn_items.pop(0)()
            if i < len(pslots):
                for (kt, eta) in pslots[i]:
                    if not pre:
                        pre = pv_prep(pa, pslot, paccs)
                    pv_tile(pa, pg, eta, kt, pre[0], oacc)
                    done[eta] = done.get(eta, 0) + 1
                    if done[eta] == 3:
                        pv_fin(pa, pg, eta, pre[1], oacc)
            if early and n >= len(steps) - KE + 1 and i == 5:
                a_ = early.pop(0)
                p3_block(a_, a_ % 2)
        prev = (a, g, n % 2, accs) if n < len(steps) else None
    assert not ffn_items
    for a_ in early:
        p3_block(a_, a_ % 2)

    def safe_attention():
        rowh = lax.broadcasted_iota(I32, (128, 128), 0) // 16
        kj = lax.broadcasted_iota(I32, (128, 128), 0)
        qj = lax.broadcasted_iota(I32, (128, 128), 1)

        def body(t, c):
            a = t // 32
            h = t % 32
            g = h // 8
            qt = qt_v[a, pl.ds(pl.multiple_of(g * 128, 128), 128), :]
            rhs = jnp.where(rowh == h % 8, qt, jnp.zeros_like(qt))
            ss = []
            kbs = []
            for kt in range(3):
                kb = a - 2 + kt
                kbc = jnp.maximum(kb, 0)
                kbs.append(kbc)
                kw = k_v[g, pl.ds(pl.multiple_of(kbc * 128, 128), 128), :]
                sc = jnp.dot(kw, rhs, preferred_element_type=F32)
                d = (a - kb) * 128 + qj - kj
                ss.append(jnp.where((kb >= 0) & (d >= 0) & (d < 256), sc, -1e9 * LOG2E))
            m = jnp.max(jnp.maximum(jnp.maximum(ss[0], ss[1]), ss[2]), axis=0, keepdims=True)
            l = None
            o = None
            for kt in range(3):
                p = jnp.exp2(ss[kt] - m)
                lt = jnp.sum(p, axis=0, keepdims=True)
                l = lt if l is None else l + lt
                vt = vt_v[kbs[kt], pl.ds(pl.multiple_of(h * 16, 16), 16), :]
                ot = jnp.dot(vt, p.astype(BF), preferred_element_type=F32)
                o = ot if o is None else o + ot
            ot_v[a, pl.ds(pl.multiple_of(h * 16, 16), 16), :] = (o / l).astype(BF)
            return c

        lax.fori_loop(0, NQ * 32, body, 0)
        for a_ in range(KE):
            out_copy(a_).wait()

        def redo(a_, c):
            p3_block(a_, 0)
            return c

        lax.fori_loop(0, KE, redo, 0)

    lo_ok = jnp.min(lrange[0]) >= L_LO
    hi_ok = jnp.max(lrange[1]) <= L_HI
    pl.when(jnp.logical_not(jnp.logical_and(lo_ok, hi_ok)))(safe_attention)

    n3 = (NQ - KE) // 2

    def p3_body(i, c):
        for j in range(n3):
            p3_block(KE + i * n3 + j, j % 2)
        return c

    lax.fori_loop(0, 2, p3_body, 0)
    for a in range(NQ):
        out_copy(a).wait()


@jax.jit
def pallas_parallel_sum__sliding_block__moe_arch_mod__prompt_kernel(
    A_x, A_wqkv, A_wo, B_x, B_w_r, B_w_gate, B_w_up, B_w_down,
):
    del B_x
    hbm = pl.BlockSpec(memory_space=pltpu.HBM)
    out = pl.pallas_call(
        _kernel,
        out_shape=jax.ShapeDtypeStruct((S, D), BF),
        in_specs=[hbm, hbm, hbm, pl.BlockSpec(memory_space=pltpu.VMEM), hbm, hbm, hbm],
        out_specs=hbm,
        scratch_shapes=[
            pltpu.VMEM((S, D), BF),
            pltpu.VMEM((D, 3 * D), BF),
            pltpu.VMEM((D, D), BF),
            pltpu.VMEM((F, D), BF),
            pltpu.VMEM((F, D), BF),
            pltpu.VMEM((F, D), BF),
            pltpu.VMEM((S, 128), F32),
            pltpu.VMEM((S, 128), F32),
            pltpu.VMEM((12, 8, 128), F32),
            pltpu.VMEM((16, D), F32),
            pltpu.VMEM((4, S, 128), BF),
            pltpu.VMEM((NQ, D, 128), BF),
            pltpu.VMEM((NQ, D, 128), BF),
            pltpu.VMEM((2, G, NR, 128), BF),
            pltpu.VMEM((2 * B, 128), F32),
            pltpu.VMEM((NQ, D, 128), BF),
            pltpu.VMEM((2, 128, D), BF),
            pltpu.VMEM((S, D), BF),
            pltpu.SemaphoreType.DMA((4,)),
            pltpu.SemaphoreType.DMA((7,)),
            pltpu.SemaphoreType.DMA((1,)),
        ],
        compiler_params=pltpu.CompilerParams(vmem_limit_bytes=100 * 2**20),
    )(A_x.reshape(S, D), A_wqkv, A_wo, B_w_r, B_w_gate.T, B_w_up.T, B_w_down)
    return out.reshape(1, S, D)
```

```python
import functools

import jax
import jax.numpy as jnp
import numpy as np
from jax import lax
import jax.experimental.pallas as pl
import jax.experimental.pallas.tpu as pltpu

S = 2048
D = 512
F = 1376
NF = 11
T1 = 512
N1 = S // T1
NQ = S // 128
LOG2E = 1.4426950408889634
QSCALE = 0.25 * LOG2E
G = 8
B = 128 // G
NR = 256 + B
LG = 3
CUTS = (0, 112, 192, NR)
ORDER = (0, 1, 2, 3, 8, 9, 10, 11, 4, 5, 6, 7)
KE = 2
L_LO = (127 - 40) << 23
L_HI = (127 + 40) << 23
BF = jnp.bfloat16
F32 = jnp.float32
I32 = jnp.int32
NT = (((1,), (1,)), ((), ()))


def _np_bf16(v):
    u = np.array([v], np.float32).view(np.uint32)
    u = (u + 0x7FFF + ((u >> 16) & 1)) & 0xFFFF0000
    return float(u.astype(np.uint32).view(np.float32)[0])


EPS_B = _np_bf16(1e-5)


def bi(x):
    return pltpu.bitcast(x, I32)


def bb(x):
    return pltpu.bitcast(x, BF)


def _rb(x):
    return x.astype(BF).astype(F32)


def _kernel(x_hbm, wqkv_hbm, wo_hbm, wr_hbm, wg_hbm, wu_hbm, wd_hbm, out_hbm,
            x_v, wqkv_v, wo_v, wr_v, wg_v, wu_v, wd_v,
            mb_v, ri_v, cs_v, upd_v, k_v, qt_v, vt_v, pbuf, bias_v, ot_v, on_v, out_v,
            x_sem, w_sem, o_sem):
    XCH = [(0, 256), (256, 256), (T1, T1), (2 * T1, S - 2 * T1)]

    def x_copy(j):
        r = pl.ds(*XCH[j])
        return pltpu.make_async_copy(x_hbm.at[r], x_v.at[r], x_sem.at[j])

    def wq_copy(j):
        c = pl.ds(j * D, D)
        return pltpu.make_async_copy(wqkv_hbm.at[:, c], wqkv_v.at[:, c], w_sem.at[j])

    wo_copy = pltpu.make_async_copy(wo_hbm, wo_v, w_sem.at[3])
    ffn_copies = [
        pltpu.make_async_copy(wg_hbm, wg_v, w_sem.at[4]),
        pltpu.make_async_copy(wu_hbm, wu_v, w_sem.at[5]),
        pltpu.make_async_copy(wd_hbm, wd_v, w_sem.at[6]),
    ]
    wr_copy = pltpu.make_async_copy(wr_hbm, wr_v, w_sem.at[7])
    x_copy(0).start()
    wr_copy.start()
    wq_copy(0).start()
    x_copy(1).start()
    wq_copy(1).start()
    wq_copy(2).start()
    x_copy(2).start()

    ki = k_v.bitcast(I32)
    qti = qt_v.bitcast(I32)
    pbi = pbuf.bitcast(I32)
    vti = vt_v.bitcast(I32)

    x_copy(0).wait()
    wr_copy.wait()
    wr = wr_v[...].astype(F32).reshape(1, D)
    swr = jnp.sum(wr, axis=1, keepdims=True)

    def row_stats(x):
        mean = jnp.mean(x, axis=1, keepdims=True)
        c = x - mean
        var = jnp.mean(c * c, axis=1, keepdims=True)
        mb = _rb(mean)
        sd = _rb(jnp.sqrt(_rb(_rb(var) + EPS_B)))
        return mb, sd

    def stats(r0, nr, best_m, best_i):
        r = pl.ds(r0, nr)
        x = x_v[r, :].astype(F32)
        mb, sd = row_stats(x)
        ri = 1.0 / sd
        mb_v[r, :] = jnp.broadcast_to(mb * ri, (nr, 128))
        ri_v[r, :] = jnp.broadcast_to(ri, (nr, 128))
        rr = _rb((jnp.sum(x * wr, axis=1, keepdims=True) - mb * swr) * ri)
        m = jnp.max(rr, axis=0, keepdims=True)
        rows = lax.broadcasted_iota(I32, (nr, 1), 0) + r0
        idx = jnp.min(jnp.where(rr == m, rows, S), axis=0, keepdims=True)
        better = m > best_m
        return jnp.where(better, m, best_m), jnp.where(better, idx, best_i)

    def colsum(ns):
        for n in ns:
            cs_v[n] = jnp.dot(jnp.ones((16, D), BF), wqkv_v[:, n * 128:(n + 1) * 128],
                              preferred_element_type=F32)[0:8]

    def project(b0, nb, ns):
        r = pl.ds(b0 * 128 if isinstance(b0, int) else pl.multiple_of(b0 * 128, 128), nb * 128)
        accs = {n: jnp.dot(x_v[r, :], wqkv_v[:, n * 128:(n + 1) * 128], preferred_element_type=F32) for n in ns}
        mb = mb_v[r, :]
        ri = ri_v[r, :]
        for n in ns:
            cs = jnp.broadcast_to(cs_v[n, 0:1, :], (nb * 128, 128))
            y = accs[n] * ri - mb * cs
            if n < 4:
                y = y * QSCALE
                for j in range(nb):
                    qt_v[b0 + j, n * 128:(n + 1) * 128, :] = y[j * 128:(j + 1) * 128].T.astype(BF)
            elif n < 8:
                k_v[n - 4, r, :] = y.astype(BF)
            else:
                for j in range(nb):
                    vt_v[b0 + j, (n - 8) * 128:(n - 7) * 128, :] = y[j * 128:(j + 1) * 128].T.astype(BF)

    QN, KN, VN = range(0, 4), range(4, 8), range(8, 12)
    carry = (jnp.full((1, 1), -jnp.inf, F32), jnp.full((1, 1), S - 1, I32))
    carry = stats(0, 256, *carry)
    wq_copy(0).wait()
    x_copy(3).start()
    wo_copy.start()
    colsum(QN)
    project(0, 2, QN)
    x_copy(1).wait()
    wq_copy(1).wait()
    colsum(KN)
    carry = stats(256, 256, *carry)
    project(0, 2, KN)
    project(2, 2, list(QN) + list(KN))
    wq_copy(2).wait()
    x_copy(2).wait()
    for c in ffn_copies:
        c.start()
    colsum(VN)
    project(0, 4, VN)
    carry = stats(T1, T1, *carry)
    x_copy(3).wait()

    def p1_body(i, carry):
        project(i * 4, 4, ORDER)
        return stats(pl.multiple_of(jnp.minimum(i + 1, N1 - 1) * T1, T1), T1, *carry)

    best_m, best_i = lax.fori_loop(1, N1, p1_body, carry)

    for c in ffn_copies:
        c.wait()
    wo_copy.wait()
    idx = jnp.clip(jnp.max(best_i), 0, S - 1)
    blk = pl.multiple_of((idx // 16) * 16, 16)
    row_sel = lax.broadcasted_iota(I32, (16, 1), 0) == (idx - blk)
    xr = x_v[pl.ds(blk, 16), :].astype(F32)
    mbr, sdr = row_stats(xr)
    xs = jnp.where(row_sel, _rb(xr - mbr) / sdr, 0.0).astype(BF)
    ffn = {}

    def ffn_gate(n):
        r = pl.ds(n * 128, min(128, F - n * 128))
        ffn['g', n] = _rb(lax.dot_general(xs, wg_v[r, :], NT, preferred_element_type=F32))

    def ffn_up(n):
        r = pl.ds(n * 128, min(128, F - n * 128))
        u_ = _rb(lax.dot_general(xs, wu_v[r, :], NT, preferred_element_type=F32))
        g_ = ffn['g', n]
        sg = _rb(g_ * _rb(jax.nn.sigmoid(g_)))
        ffn['h', n] = (sg * u_).astype(BF)

    def ffn_down(n):
        r = pl.ds(n * 128, min(128, F - n * 128))
        y = jnp.dot(ffn['h', n], wd_v[r, :], preferred_element_type=F32)
        ffn['y'] = y if n == 0 else ffn['y'] + y
        if n == NF - 1:
            rs = _rb(jax.nn.sigmoid(best_m))
            upd_v[...] = jnp.where(row_sel, _rb(_rb(ffn['y']) * rs), 0.0)

    ffn_items = []
    for n in range(NF):
        ffn_items += [functools.partial(ffn_gate, n), functools.partial(ffn_up, n)]
        if n > 0:
            ffn_items.append(functools.partial(ffn_down, n - 1))
    ffn_items.append(functools.partial(ffn_down, NF - 1))

    lane = lax.broadcasted_iota(I32, (B, 128), 1)
    row = lax.broadcasted_iota(I32, (B, 128), 0)
    qi = lane & (B - 1)
    bias_v[0:B] = jnp.where(row > qi, 0.0, -jnp.inf)
    bias_v[B:2 * B] = jnp.where(row <= qi, 0.0, -jnp.inf)

    def lgrp(r):
        return lax.broadcasted_iota(I32, (r, 128), 1) // B

    gm = [jnp.where(lgrp(8) == p, -1, 0).astype(I32) for p in range(G)]

    def bitmask(r, k):
        return ((lgrp(r) >> k) & 1) == 0

    def zrows(n):
        return jnp.zeros((n, 128), I32)

    def stage(X0, X1, k):
        sh = (B // 2) << k
        A = jnp.concatenate([X0, zrows(sh)], axis=0)
        Bm = jnp.concatenate([zrows(sh), X1], axis=0)
        m = bitmask(A.shape[0], k)
        return jnp.where(m, A, Bm), jnp.where(m, Bm, A)

    lrange = [jnp.full((1, 128), 0x7F000000, I32), jnp.zeros((1, 128), I32)]

    def qk_prep(a, g, s):
        qt = qti[a, pl.ds(g * 64, 64), :]
        parts = []
        for hp in range(8):
            p = hp ^ s
            x = qt[hp * 8:hp * 8 + 8]
            sh = ((p - s) * B) % 128
            if sh:
                x = pltpu.roll(x, sh, 1)
            parts.append(x & gm[p])
        return bb(jnp.concatenate(parts, axis=0))

    def qk_piece(a, g, s, rhs, r0, r1, slot, accs):
        base = a * 128 + s * B - 256
        r0 = max(r0, -base)
        if r0 >= r1:
            return
        kw = bb(ki[g, pl.ds((base + r0) // 2, (r1 - r0) // 2), :])
        sc = jnp.dot(kw, rhs, preferred_element_type=F32)
        acc = accs.get(s)
        for r in range(r0, r1, 16):
            sr = sc[r - r0:r - r0 + 16]
            if r < B:
                sr = sr + bias_v[r:r + 16]
            if r >= 256:
                sr = sr + bias_v[B + r - 256:B + r - 256 + 16]
            p = jnp.exp2(sr)
            t = p[0:8] + p[8:16]
            acc = t if acc is None else acc + t
            pbuf[slot, s, r:r + 16] = p.astype(BF)
        accs[s] = acc

    def pv_prep(a, slot, accs):
        idx = {}
        for s in range(G):
            base = a * 128 + s * B - 256
            if base >= 0:
                idx[(s, 0)] = pbi[slot, s, 0:NR // 2]
            else:
                z = min(-base, NR)
                idx[(s, 0)] = jnp.concatenate(
                    [zrows(z // 2), pbi[slot, s, z // 2:NR // 2]], axis=0)
        lidx = {(s, 0): jnp.sum(accs[s], axis=0, keepdims=True) for s in range(G)}
        for s in range(G):
            lb = pltpu.bitcast(lidx[(s, 0)], I32)
            lrange[0] = jnp.minimum(lrange[0], lb)
            lrange[1] = jnp.maximum(lrange[1], lb)
        for k in range(LG):
            nidx = {}
            nl = {}
            for sh in range(G >> (k + 1)):
                for c in range(1 << k):
                    Y0, Y1 = stage(idx[(2 * sh, c)], idx[(2 * sh + 1, c)], k)
                    nidx[(sh, c)] = Y0
                    nidx[(sh, c | (1 << k))] = Y1
                    m1 = bitmask(1, k)
                    la, lb = lidx[(2 * sh, c)], lidx[(2 * sh + 1, c)]
                    nl[(sh, c)] = jnp.where(m1, la, lb)
                    nl[(sh, c | (1 << k))] = jnp.where(m1, lb, la)
            idx = nidx
            lidx = nl
        return idx, lidx

    def pv_tile(a, g, eta, kt, W, oacc):
        key0 = a * 128 - 256 + kt * 128
        if key0 < 0:
            return
        h = g * 8 + eta
        vt = bb(vti[key0 // 128, pl.ds(h * 8, 8), :])
        o = jnp.dot(vt, bb(W[(0, eta)][kt * 64:(kt + 1) * 64]), preferred_element_type=F32)
        oacc[eta] = o if eta not in oacc else oacc[eta] + o

    def pv_fin(a, g, eta, lidx, oacc):
        h = g * 8 + eta
        l = lidx[(0, eta)]
        r0 = pltpu.reciprocal(l, approx=True)
        r1 = r0 * (2.0 - l * r0)
        ob = bi((oacc[eta] * r1).astype(BF))
        for k in range(LG):
            if (eta >> k) & 1:
                d = B << k
                if d == 64:
                    ob = pltpu.roll(ob, 64, 1)
                else:
                    ob = jnp.where(bitmask(8, k), pltpu.roll(ob, 128 - d, 1), pltpu.roll(ob, d, 1))
        ot_v[a, pl.ds(h * 16, 16), :] = bb(ob)

    def out_copy(a):
        r = pl.ds(a * 128 if isinstance(a, int) else pl.multiple_of(a * 128, 128), 128)
        return pltpu.make_async_copy(out_v.at[r], out_hbm.at[r], o_sem.at[0])

    def p3_block(a, par):
        r0 = a * 128 if isinstance(a, int) else pl.multiple_of(a * 128, 128)
        r = pl.ds(r0, 128)
        on_v[par] = ot_v[a].T
        att = jnp.dot(on_v[par], wo_v[...], preferred_element_type=F32)
        x = x_v[r, :].astype(F32)
        ri = jnp.concatenate([ri_v[r, :]] * 4, axis=1)
        mb = jnp.concatenate([mb_v[r, :]] * 4, axis=1)
        ups = jnp.concatenate([jnp.where(r0 + 16 * t == blk, upd_v[...], 0.0) for t in range(8)], axis=0)
        out_v[r, :] = (att + (x + (x * ri - mb)) + ups).astype(BF)
        out_copy(a).start()

    steps = [(a, g) for a in range(NQ) for g in range(4)]
    early = list(range(KE))
    prev = None
    for n in range(len(steps) + 1):
        qslots = []
        pslots = []
        accs = {}
        rh = {}
        pre = []
        oacc = {}
        done = {}
        if n < len(steps):
            a, g = steps[n]
            for ss in ([0, 1, 2, 3], [4, 5, 6, 7]):
                for pi in range(len(CUTS) - 1):
                    qslots.append((ss, CUTS[pi], CUTS[pi + 1]))
        if prev is not None:
            pa, pg, pslot, paccs = prev
            tiles = [(kt, e) for e0 in (0, 4) for kt in range(3) for e in range(e0, e0 + 4)]
            pslots = [tiles[i:i + 4] for i in range(0, len(tiles), 4)]
        for i in range(max(len(qslots), len(pslots))):
            if i < len(qslots):
                ss, r0, r1 = qslots[i]
                for s_ in ss:
                    if s_ not in rh:
                        rh[s_] = qk_prep(a, g, s_)
                    qk_piece(a, g, s_, rh[s_], r0, r1, n % 2, accs)
            if ffn_items and i == 0:
                ffn_items.pop(0)()
            if i < len(pslots):
                for (kt, eta) in pslots[i]:
                    if not pre:
                        pre = pv_prep(pa, pslot, paccs)
                    pv_tile(pa, pg, eta, kt, pre[0], oacc)
                    done[eta] = done.get(eta, 0) + 1
                    if done[eta] == 3:
                        pv_fin(pa, pg, eta, pre[1], oacc)
            if early and n >= len(steps) - KE + 1 and i == 5:
                a_ = early.pop(0)
                p3_block(a_, a_ % 2)
        prev = (a, g, n % 2, accs) if n < len(steps) else None
    assert not ffn_items
    for a_ in early:
        p3_block(a_, a_ % 2)

    def safe_attention():
        rowh = lax.broadcasted_iota(I32, (128, 128), 0) // 16
        kj = lax.broadcasted_iota(I32, (128, 128), 0)
        qj = lax.broadcasted_iota(I32, (128, 128), 1)

        def body(t, c):
            a = t // 32
            h = t % 32
            g = h // 8
            qt = qt_v[a, pl.ds(pl.multiple_of(g * 128, 128), 128), :]
            rhs = jnp.where(rowh == h % 8, qt, jnp.zeros_like(qt))
            ss = []
            kbs = []
            for kt in range(3):
                kb = a - 2 + kt
                kbc = jnp.maximum(kb, 0)
                kbs.append(kbc)
                kw = k_v[g, pl.ds(pl.multiple_of(kbc * 128, 128), 128), :]
                sc = jnp.dot(kw, rhs, preferred_element_type=F32)
                d = (a - kb) * 128 + qj - kj
                ss.append(jnp.where((kb >= 0) & (d >= 0) & (d < 256), sc, -1e9 * LOG2E))
            m = jnp.max(jnp.maximum(jnp.maximum(ss[0], ss[1]), ss[2]), axis=0, keepdims=True)
            l = None
            o = None
            for kt in range(3):
                p = jnp.exp2(ss[kt] - m)
                lt = jnp.sum(p, axis=0, keepdims=True)
                l = lt if l is None else l + lt
                vt = vt_v[kbs[kt], pl.ds(pl.multiple_of(h * 16, 16), 16), :]
                ot = jnp.dot(vt, p.astype(BF), preferred_element_type=F32)
                o = ot if o is None else o + ot
            ot_v[a, pl.ds(pl.multiple_of(h * 16, 16), 16), :] = (o / l).astype(BF)
            return c

        lax.fori_loop(0, NQ * 32, body, 0)
        for a_ in range(KE):
            out_copy(a_).wait()

        def redo(a_, c):
            p3_block(a_, 0)
            return c

        lax.fori_loop(0, KE, redo, 0)

    lo_ok = jnp.min(lrange[0]) >= L_LO
    hi_ok = jnp.max(lrange[1]) <= L_HI
    pl.when(jnp.logical_not(jnp.logical_and(lo_ok, hi_ok)))(safe_attention)

    n3 = (NQ - KE) // 2

    def p3_body(i, c):
        for j in range(n3):
            p3_block(KE + i * n3 + j, j % 2)
        return c

    lax.fori_loop(0, 2, p3_body, 0)
    for a in range(NQ):
        out_copy(a).wait()


@jax.jit
def pallas_parallel_sum__sliding_block__moe_arch_mod__prompt_kernel(
    A_x, A_wqkv, A_wo, B_x, B_w_r, B_w_gate, B_w_up, B_w_down,
):
    del B_x
    hbm = pl.BlockSpec(memory_space=pltpu.HBM)
    out = pl.pallas_call(
        _kernel,
        out_shape=jax.ShapeDtypeStruct((S, D), BF),
        in_specs=[hbm] * 7,
        out_specs=hbm,
        scratch_shapes=[
            pltpu.VMEM((S, D), BF),
            pltpu.VMEM((D, 3 * D), BF),
            pltpu.VMEM((D, D), BF),
            pltpu.VMEM((D,), BF),
            pltpu.VMEM((F, D), BF),
            pltpu.VMEM((F, D), BF),
            pltpu.VMEM((F, D), BF),
            pltpu.VMEM((S, 128), F32),
            pltpu.VMEM((S, 128), F32),
            pltpu.VMEM((12, 8, 128), F32),
            pltpu.VMEM((16, D), F32),
            pltpu.VMEM((4, S, 128), BF),
            pltpu.VMEM((NQ, D, 128), BF),
            pltpu.VMEM((NQ, D, 128), BF),
            pltpu.VMEM((2, G, NR, 128), BF),
            pltpu.VMEM((2 * B, 128), F32),
            pltpu.VMEM((NQ, D, 128), BF),
            pltpu.VMEM((2, 128, D), BF),
            pltpu.VMEM((S, D), BF),
            pltpu.SemaphoreType.DMA((4,)),
            pltpu.SemaphoreType.DMA((8,)),
            pltpu.SemaphoreType.DMA((1,)),
        ],
        compiler_params=pltpu.CompilerParams(vmem_limit_bytes=100 * 2**20),
    )(A_x.reshape(S, D), A_wqkv, A_wo, B_w_r, B_w_gate.T, B_w_up.T, B_w_down)
    return out.reshape(1, S, D)
```
